```python
import os as _os
_os.environ.setdefault('JAX_PLATFORMS', 'cpu')
import jax
import jax.numpy as jnp

def _softmax(x, axis=-1):
    return jax.nn.softmax(x, axis=axis)

def _gelu(x):
    return jax.nn.gelu(x, approximate=True)

def _silu(x):
    return jax.nn.silu(x)

def _sigmoid(x):
    return jax.nn.sigmoid(x)

def _layernorm(x, axis=-1, eps=1e-05):
    m = jnp.mean(x, axis=axis, keepdims=True)
    v = jnp.var(x, axis=axis, keepdims=True)
    return (x - m) / jnp.sqrt(v + eps)

def _scatter_add(tgt, idx, src, axis=0):
    return tgt.at[idx].add(src)

def _segment_sum(src, seg, n):
    return jax.ops.segment_sum(src, seg, n)

class _Rng:

    def __init__(self, key):
        self._k = key

    def _next(self):
        self._k, sub = jax.random.split(self._k)
        return sub

    def normal(self, shape):
        return jax.random.normal(self._next(), shape, dtype=jnp.bfloat16)

    def randint(self, lo, hi, shape):
        return jax.random.randint(self._next(), shape, lo, hi, dtype=jnp.int32)

    def uniform(self, shape, lo=0.0, hi=1.0):
        return jax.random.uniform(self._next(), shape, jnp.bfloat16, lo, hi)

    def permutation(self, n):
        return jax.random.permutation(self._next(), n)
kernel_name = 'adaLN_cond__linear_kernel_hedgehog__geglu_ffn__prompt'

def setup_inputs():
    _rng = _Rng(jax.random.key(int.from_bytes(__import__("os").urandom(4), "little")))
    _w = lambda a: (lambda t: t.astype(jnp.bfloat16) if jnp.issubdtype(t.dtype, jnp.floating) else t)(jnp.asarray(a))

    def _A_setup():
        B, S, D, H = (1, 2048, 512, 32)
        Dh = D // H
        return {'x': _w((lambda *s: _rng.normal(s) * 0.05)(B, S, D)), 'wqkv': _w((lambda *s: _rng.normal(s) * 0.4)(D, 3 * D)), 'w_phi': _w((lambda *s: _rng.normal(s) * 0.4)(H, Dh, Dh) * Dh ** (-0.5)), 'wo': _w((lambda *s: _rng.normal(s) * 0.05)(D, D))}
    _A_in = _A_setup()

    def _B_setup():
        B, S, D, F = (1, 2048, 512, 1792)
        return {'x': _w((lambda *s: _rng.normal(s) * 0.05)(B, S, D)), 'w_gate': _w((lambda *s: _rng.normal(s) * 0.05)(D, F)), 'w_up': _w((lambda *s: _rng.normal(s) * 0.05)(D, F)), 'w_down': _w((lambda *s: _rng.normal(s) * 0.05)(F, D))}
    _B_in = _B_setup()
    return {'A_x': _A_in['x'], 'A_wqkv': _A_in['wqkv'], 'A_w_phi': _A_in['w_phi'], 'A_wo': _A_in['wo'], 'B_x': _B_in['x'], 'B_w_gate': _B_in['w_gate'], 'B_w_up': _B_in['w_up'], 'B_w_down': _B_in['w_down'], 'c': _w((lambda *s: _rng.normal(s) * 0.05)(1, 512) * 8.0), 'w_mod': _w((lambda *s: _rng.normal(s) * 0.05)(512, 6 * 512) * 512 ** (-0.5) * 8.0)}

def reference(A_x, A_wqkv, A_w_phi, A_wo, B_x, B_w_gate, B_w_up, B_w_down, c, w_mod):

    def _A_ref(x, wqkv, w_phi, wo):
        B, S, D = x.shape
        H = 32
        Dh = D // H
        qkv = (lambda x, *d: x.transpose(*d))((x @ wqkv).reshape(B, S, 3, H, Dh), 2, 0, 3, 1, 4)
        q, k, v = (qkv[0], qkv[1], qkv[2])
        pq = jnp.einsum('bhsd,hdf->bhsf', q, w_phi)
        pk = jnp.einsum('bhsd,hdf->bhsf', k, w_phi)
        phi_q = jnp.concatenate([_softmax(pq, axis=-1), _softmax(-pq, axis=-1)], axis=-1)
        phi_k = jnp.concatenate([_softmax(pk, axis=-1), _softmax(-pk, axis=-1)], axis=-1)
        kv = jnp.einsum('bhsf,bhsd->bhfd', phi_k, v)
        z = jnp.einsum('bhsf->bhf', phi_k)
        num = jnp.einsum('bhqf,bhfd->bhqd', phi_q, kv)
        den = jnp.einsum('bhqf,bhf->bhq', phi_q, z)[..., None] + 1e-06
        o = num / den
        return (lambda x, *d: x.transpose(*d))(o, 0, 2, 1, 3).reshape(B, S, D) @ wo

    def _B_ref(x, w_gate, w_up, w_down):
        return _gelu(x @ w_gate) * (x @ w_up) @ w_down
    x = A_x
    mod = (_silu(c) @ w_mod).reshape(c.shape[0], 6, 1, -1)
    sa, ca, ga, sb, cb, gb = (mod[:, 0].copy(), mod[:, 1].copy(), mod[:, 2].copy(), mod[:, 3].copy(), mod[:, 4].copy(), mod[:, 5].copy())
    h = _layernorm(x, axis=-1) * (1 + ca) + sa
    x = x + ga * _A_ref(h, A_wqkv, A_w_phi, A_wo)
    h = _layernorm(x, axis=-1) * (1 + cb) + sb
    x = x + gb * _B_ref(h, B_w_gate, B_w_up, B_w_down)
    return x
```

```python
import jax
import jax.numpy as jnp
from jax import lax
import jax.experimental.pallas as pl
import jax.experimental.pallas.tpu as pltpu

S, D, H, DH, F = 2048, 512, 32, 16, 1792
G = 4
T = 512
NT = S // T
FC = 256
LOG2E = 1.4426950408889634
GC = 0.7978845608028654
F32, BF16 = jnp.float32, jnp.bfloat16
NT_DIMS = (((1,), (1,)), ((), ()))
TN_DIMS = (((0,), (0,)), ((), ()))


def _dot(a, b, dims=(((1,), (0,)), ((), ()))):
    return lax.dot_general(a, b, dims, preferred_element_type=F32)


def _ln(x):
    m = jnp.mean(x, axis=-1, keepdims=True)
    xc = x - m
    v = jnp.mean(xc * xc, axis=-1, keepdims=True)
    return xc * lax.rsqrt(v + 1e-5)


def _tree(op, xs):
    xs = list(xs)
    while len(xs) > 1:
        xs = [op(xs[i], xs[i + 1]) for i in range(0, len(xs), 2)]
    return xs[0]


def _feat(p):
    rows = [p[f * 8:(f + 1) * 8] for f in range(DH)]
    mx = _tree(jnp.maximum, rows)
    mn = _tree(jnp.minimum, rows)
    ep = [jnp.exp2(r - mx) for r in rows]
    en = [jnp.exp2(mn - r) for r in rows]
    return ep, en, _tree(jnp.add, ep), _tree(jnp.add, en)


def _kernel(x_hbm, wqkv_hbm, wphi_ref, wo_hbm, wg_hbm, wu_hbm, wd_hbm, c_v, wmod_hbm, o_hbm,
            x_v, wqkv_v, wo_v, wg_v, wu_v, wd_v, wmod_v, o_v,
            h_v, wqk_v, mod_v, kv_v, kvt_v, zb_v, phi_v, v_v, pq_v, x1_v, h2_v, act_v, sems):
    def cp(src, dst, i):
        return pltpu.make_async_copy(src, dst, sems.at[i])

    c_mod = [cp(wmod_hbm.at[:, pl.ds(s, n)], wmod_v.at[:, pl.ds(s, n)], i)
             for i, (s, n) in enumerate([(0, D), (D, D), (2 * D, 4 * D)])]
    c_w = [cp(wqkv_hbm.at[:, pl.ds(i * D, D)], wqkv_v.at[:, pl.ds(i * D, D)], 3 + i) for i in range(3)]
    c_ffn = [cp(wo_hbm, wo_v, 6), cp(wg_hbm, wg_v, 7), cp(wu_hbm, wu_v, 8), cp(wd_hbm, wd_v, 9)]

    def c_x(i):
        return cp(x_hbm.at[pl.ds(i * T, T)], x_v.at[pl.ds(i * T, T)], 10 + i)

    def c_o(i):
        return cp(o_v.at[pl.ds(i * T, T)], o_hbm.at[pl.ds(i * T, T)], 10 + NT + i)

    for d in [c_x(0), c_w[1], c_mod[1], c_mod[0]]:
        d.start()
    C = 512
    NC = T // C
    c_x(0).wait()
    x1_v[0] = _ln(x_v[0:T, :].astype(F32))

    def iota(shape, ax):
        return lax.broadcasted_iota(jnp.int32, shape, ax)

    et = (iota((128, DH), 0) // 8 == iota((128, DH), 1)).astype(F32).astype(BF16)
    wl = jnp.concatenate([wphi_ref[d * DH:(d + 1) * DH, :] for d in range(DH)], axis=1)
    rr, cc = iota((128, D), 0), iota((128, D), 1)
    rep_ = jnp.where(rr % 8 == cc % 8, _dot(et, wl), 0.0)
    sel = ((rr // DH == cc % 8) & (rr % DH == cc // H)).astype(F32).astype(BF16)
    pm = [_dot(jnp.where((cc % H) // 8 == g, rep_, 0.0).astype(BF16), sel, NT_DIMS).astype(BF16)
          for g in range(G)]

    def fold(j):
        for g in range(G):
            w = wqkv_v[:, j * D + g * 128:j * D + (g + 1) * 128]
            wqk_v[j, g * 128:(g + 1) * 128, :] = (_dot(pm[g], w, NT_DIMS) * LOG2E).astype(BF16)

    c_w[1].wait()
    fold(1)
    cv = c_v[...].astype(F32)
    sc = jnp.broadcast_to(cv * jax.nn.sigmoid(cv), (16, D)).astype(BF16)

    def mods(s, n):
        mod_v[:, s:s + n] = _dot(sc, wmod_v[:, s:s + n])

    c_mod[1].wait()
    mods(D, D)
    c_mod[0].wait()
    mods(0, D)
    for d in [c_w[2]] + [c_x(i) for i in range(1, NT)] + [c_w[0], c_mod[2]] + c_ffn:
        d.start()

    zs = [None] * G

    def ln1(i, t):
        r = pl.ds(i * T + t * C, C)
        h_v[r, :] = ((x1_v[0, r, :] if i == 0 else _ln(x_v[r, :].astype(F32))) * (1.0 + mod_v[0:1, D:2 * D])
                     + mod_v[0:1, 0:D]).astype(BF16)

    def kfeat(i, t):
        r = pl.ds(i * T + t * C, C)
        pk = _dot(wqk_v[1], h_v[r, :], NT_DIMS)
        for g in range(G):
            ep, en, sp, sn = _feat(pk[g * 128:(g + 1) * 128])
            rp, rn = 1.0 / sp, 1.0 / sn
            phi = jnp.concatenate([e * rp for e in ep] + [e * rn for e in en], axis=0)
            zs[g] = phi if zs[g] is None else zs[g] + phi
            phi_v[i % 2, g, :, t * C:(t + 1) * C] = phi.astype(BF16)

    def vproj(i, t):
        r = pl.ds(i * T + t * C, C)
        v_v[i % 2, t * C:(t + 1) * C, :] = _dot(h_v[r, :], wqkv_v[:, 2 * D:3 * D]).astype(BF16)

    def kvacc(i, g):
        kv = _dot(phi_v[i % 2, g], v_v[i % 2, :, g * 128:(g + 1) * 128])
        kv_v[g] = kv if i == 0 else kv_v[g] + kv

    def qproj(i, t):
        pq_v[:, t * C:(t + 1) * C] = _dot(wqk_v[0], h_v[pl.ds(i * T + t * C, C), :], NT_DIMS)

    def qfeat(t):
        for g in range(G):
            ep, en, sp, sn = _feat(pq_v[g * 128:(g + 1) * 128, t * C:(t + 1) * C])
            rp, rn = 1.0 / sp, 1.0 / sn
            dp = _tree(jnp.add, [ep[f] * zb_v[g, f * 8:(f + 1) * 8] for f in range(DH)])
            dn = _tree(jnp.add, [en[f] * zb_v[g, 128 + f * 8:128 + (f + 1) * 8] for f in range(DH)])
            rd = 1.0 / (dp * rp + dn * rn + 1e-6)
            rp, rn = rp * rd, rn * rd
            phi_v[0, g, :, t * C:(t + 1) * C] = jnp.concatenate(
                [e * rp for e in ep] + [e * rn for e in en], axis=0).astype(BF16)

    def attn_out(i):
        ot = jnp.concatenate([_dot(kvt_v[g], phi_v[0, g]).astype(BF16) for g in range(G)], axis=0)
        att = _dot(ot, wo_v[...], TN_DIMS)
        x1 = x_v[pl.ds(pl.multiple_of(i * T, T), T), :].astype(F32) + mod_v[0:1, 2 * D:3 * D] * att
        x1_v[0] = x1
        h2_v[0] = (_ln(x1) * (1.0 + mod_v[0:1, 4 * D:5 * D])
                       + mod_v[0:1, 3 * D:4 * D]).astype(BF16)

    for t in range(NC):
        ln1(0, t)
    for i in range(NT):
        if i == 1:
            for j in range(2, NT):
                c_x(j).wait()
        if i == 3:
            c_w[0].wait()
            fold(0)
        for t in range(NC):
            kfeat(i, t)
            if i == 0 and t == NC - 1:
                c_w[2].wait()
                c_x(1).wait()
                for u in range(NC):
                    vproj(0, u)
                    ln1(1, u)
            if i > 0:
                vproj(i, t)
                [kvacc(i - 1, u) for u in range(G)]
                if i + 1 < NT:
                    ln1(i + 1, t)
    for t in range(NC):
        [kvacc(NT - 1, u) for u in range(G)]
    for d in c_ffn:
        d.wait()
    kmask = (iota((128, 256), 0) // DH) == (iota((128, 256), 1) % 8)
    for g in range(G):
        kvt_v[g] = jnp.where(kmask, kv_v[g].T, 0.0).astype(BF16)
        zb_v[g] = jnp.broadcast_to(jnp.sum(zs[g], axis=-1, keepdims=True), (256, 512))
    c_mod[2].wait()
    for t in range(4):
        mods((2 + t) * D, D)

    def phase2(i):
        r = pl.ds(pl.multiple_of(i * T, T), T)
        pq_v[...] = _dot(wqk_v[0], h_v[r, :], NT_DIMS)
        for g in range(G):
            qfeat(g) if g == 0 else None
        attn_out(i)
        h2 = h2_v[0]
        for s in range(0, F, FC):
            a = _dot(h2, wg_v[:, s:s + FC])
            b = _dot(h2, wu_v[:, s:s + FC])
            th = jnp.tanh(a * (GC + (GC * 0.044715) * (a * a)))
            ha = 0.5 * a
            act_v[:, s:s + FC] = ((ha * th + ha) * b).astype(BF16)
        y = _dot(act_v[...], wd_v[...])
        o_v[r, :] = (x1_v[0] + mod_v[0:1, 5 * D:] * y).astype(BF16)
        c_o(i).start()

    pl.loop(0, NT)(phase2)
    for i in range(NT):
        c_o(i).wait()


@jax.jit
def pallas_adaLN_cond__linear_kernel_hedgehog__geglu_ffn__prompt_kernel(
    A_x: jax.Array,
    A_wqkv: jax.Array,
    A_w_phi: jax.Array,
    A_wo: jax.Array,
    B_x: jax.Array,
    B_w_gate: jax.Array,
    B_w_up: jax.Array,
    B_w_down: jax.Array,
    c: jax.Array,
    w_mod: jax.Array,
):
    del B_x
    hbm = pl.BlockSpec(memory_space=pl.ANY)
    vmem = pl.BlockSpec(memory_space=pltpu.VMEM)
    out = pl.pallas_call(
        _kernel,
        out_shape=jax.ShapeDtypeStruct((S, D), BF16),
        in_specs=[hbm, hbm, vmem, hbm, hbm, hbm, hbm, vmem, hbm],
        out_specs=hbm,
        scratch_shapes=[
            pltpu.VMEM((S, D), BF16),
            pltpu.VMEM((D, 3 * D), BF16),
            pltpu.VMEM((D, D), BF16),
            pltpu.VMEM((D, F), BF16),
            pltpu.VMEM((D, F), BF16),
            pltpu.VMEM((F, D), BF16),
            pltpu.VMEM((D, 6 * D), BF16),
            pltpu.VMEM((S, D), BF16),
            pltpu.VMEM((S, D), BF16),
            pltpu.VMEM((2, D, D), BF16),
            pltpu.VMEM((16, 6 * D), F32),
            pltpu.VMEM((G, 256, 128), F32),
            pltpu.VMEM((G, 128, 256), BF16),
            pltpu.VMEM((G, 256, 512), F32),
            pltpu.VMEM((2, G, 256, T), BF16),
            pltpu.VMEM((2, T, D), BF16),
            pltpu.VMEM((D, T), F32),
            pltpu.VMEM((2, T, D), F32),
            pltpu.VMEM((2, T, D), BF16),
            pltpu.VMEM((T, F), BF16),
            pltpu.SemaphoreType.DMA((12 + 2 * NT,)),
        ],
        compiler_params=pltpu.CompilerParams(vmem_limit_bytes=100 * 1024 * 1024),
    )(A_x.reshape(S, D), A_wqkv, A_w_phi.transpose(1, 2, 0).reshape(DH * DH, H), A_wo, B_w_gate, B_w_up, B_w_down, c, w_mod)
    return out.reshape(A_x.shape)
```
